```python
import os as _os
_os.environ.setdefault("JAX_PLATFORMS", "cpu")
import jax
import jax.numpy as jnp

def _softmax(x, axis=-1):
    return jax.nn.softmax(x, axis=axis)
def _gelu(x):
    return jax.nn.gelu(x, approximate=True)
def _silu(x):
    return jax.nn.silu(x)
def _sigmoid(x):
    return jax.nn.sigmoid(x)
def _layernorm(x, axis=-1, eps=1e-5):
    m = jnp.mean(x, axis=axis, keepdims=True)
    v = jnp.var(x, axis=axis, keepdims=True)
    return (x - m) / jnp.sqrt(v + eps)
def _scatter_add(tgt, idx, src, axis=0):
    return tgt.at[idx].add(src)
def _segment_sum(src, seg, n):
    return jax.ops.segment_sum(src, seg, n)
class _Rng:
    def __init__(self, key):
        self._k = key
    def _next(self):
        self._k, sub = jax.random.split(self._k)
        return sub
    def normal(self, shape):
        return jax.random.normal(self._next(), shape, dtype=jnp.bfloat16)
    def randint(self, lo, hi, shape):
        return jax.random.randint(self._next(), shape, lo, hi, dtype=jnp.int32)
    def uniform(self, shape, lo=0.0, hi=1.0):
        return jax.random.uniform(self._next(), shape, jnp.bfloat16, lo, hi)
    def permutation(self, n):
        return jax.random.permutation(self._next(), n)


kernel_name = 'interleave_layers__gqa_block_cached__dense_activation_mish__decode'

def setup_inputs():
    _rng = _Rng(jax.random.key(int.from_bytes(__import__("os").urandom(4), "little")))
    _w = (lambda a: (lambda t: t.astype(jnp.bfloat16) if jnp.issubdtype(t.dtype, jnp.floating) else t)(jnp.asarray(a)))
    def _A_setup():
        B, Sq, D = 1, 1, 512
        Hq, Hkv, Sk, Dh = 32, 8, 65536, 128
        assert Hq % Hkv == 0, (Hq, Hkv)
        return {
            "x": _w((lambda *s: _rng.normal(s) * 0.05)(B, Sq, D)),
            "k_cache": _w((lambda *s: _rng.normal(s) * 1.6)(B, Hkv, Sk, Dh)),
            "v_cache": _w((lambda *s: _rng.normal(s) * 1.6)(B, Hkv, Sk, Dh)),
            "wq": _w((lambda *s: _rng.normal(s) * 1.6)(D, Hq * Dh) * (D ** -0.5)),
            "wo": _w((lambda *s: _rng.normal(s) * 1.6)(Hq * Dh, D) * ((Hq * Dh) ** -0.5)),
        }
    _A_in = _A_setup()

    def _B_setup():
        B, S, D, F = 1, 1, 512, 1792
        return {
            "x": _w((lambda *s: _rng.normal(s) * 0.05)(B, S, D)),
            "w1": _w((lambda *s: _rng.normal(s) * 0.8)(D, F) * (D ** -0.5)),
            "b1": _w((lambda *s: _rng.normal(s) * 0.8)(F)),
            "w2": _w((lambda *s: _rng.normal(s) * 0.8)(F, D) * (F ** -0.5)),
        }
    _B_in = _B_setup()

    return {
        "A_x": _A_in["x"],
        "A_k_cache": _A_in["k_cache"],
        "A_v_cache": _A_in["v_cache"],
        "A_wq": _A_in["wq"],
        "A_wo": _A_in["wo"],
        "B_x": _B_in["x"],
        "B_w1": _B_in["w1"],
        "B_b1": _B_in["b1"],
        "B_w2": _B_in["w2"],
    }

def reference(A_x, A_k_cache, A_v_cache, A_wq, A_wo, B_x, B_w1, B_b1, B_w2):
    def _A_ref(x, k_cache, v_cache, wq, wo):
        B, Sq, D = x.shape
        Hq, Dh = 32, 128
        Hkv = k_cache.shape[1]
        rep = Hq // Hkv
        q = (lambda x, *d: x.transpose(*d))((x @ wq).reshape(B, Sq, Hq, Dh), 0, 2, 1, 3)
        k = jnp.repeat(k_cache, rep, axis=1)
        v = jnp.repeat(v_cache, rep, axis=1)
        scores = jnp.einsum("bhqd,bhkd->bhqk", q, k) * (Dh ** -0.5)
        p = _softmax(scores, axis=-1)
        o = jnp.einsum("bhqk,bhkd->bhqd", p, v)
        return (lambda x, *d: x.transpose(*d))(o, 0, 2, 1, 3).reshape(B, Sq, Hq * Dh) @ wo

    def _B_ref(x, w1, b1, w2):
        h = jnp.einsum("bsd,df->bsf", x, w1) + b1
        sp = jnp.log1p(jnp.exp(-jnp.abs(h))) + jnp.where(h > 0, h, jnp.zeros_like(h))
        act = h * jnp.tanh(sp)
        return jnp.einsum("bsf,fd->bsd", act, w2)

    x = A_x
    x = x + _A_ref(_layernorm(x, axis=-1), A_k_cache, A_v_cache, A_wq, A_wo)
    x = x + _B_ref(_layernorm(x, axis=-1), B_w1, B_b1, B_w2)
    x = x + _A_ref(_layernorm(x, axis=-1), A_k_cache, A_v_cache, A_wq, A_wo)
    x = x + _B_ref(_layernorm(x, axis=-1), B_w1, B_b1, B_w2)
    return x
```

```python
import functools
import numpy as np
import jax
import jax.numpy as jnp
from jax import lax
import jax.experimental.pallas as pl
import jax.experimental.pallas.tpu as pltpu

HQ, HKV, DH, SK, D, F = 32, 8, 128, 65536, 512, 1792
REP = HQ // HKV
LOG2E = float(np.log2(np.e))
QSCALE = float(DH ** -0.5 * LOG2E)
NEG = -1e30


def _ln(x):
    m = jnp.mean(x, axis=-1, keepdims=True)
    xc = x - m
    v = jnp.mean(xc * xc, axis=-1, keepdims=True)
    return xc / jnp.sqrt(v + 1e-5)


def _dot(a, b):
    return jnp.dot(a, b, preferred_element_type=jnp.float32)


def _dot_nt(a, b):
    return lax.dot_general(a, b, (((1,), (1,)), ((), ())), preferred_element_type=jnp.float32)


def make_kernel(U=4096, S=58, no_dma=False, no_compute=False, layers=2):
    NU = HKV * SK // U
    UPG = SK // U
    assert S <= NU

    def kernel(x_hbm, k_hbm, v_hbm, wq_hbm, wo_hbm, w1_hbm, b1_hbm, w2_hbm, out_ref,
               kbuf, vbuf, wq_v, wo_v, w1_v, w2_v, x_v, b1_v, q_v, s_v, m_v, l_v, acc_v,
               ksem, vsem, wsem):
        def k_copy(u, slot):
            g = u // UPG
            c = u % UPG
            return pltpu.make_async_copy(k_hbm.at[0, g, pl.ds(c * U, U)], kbuf.at[slot], ksem.at[slot])

        def v_copy(u, slot):
            g = u // UPG
            c = u % UPG
            return pltpu.make_async_copy(v_hbm.at[0, g, pl.ds(c * U, U)], vbuf.at[slot], vsem.at[slot])

        def k_wait(slot):
            pltpu.make_async_copy(k_hbm.at[0, 0, pl.ds(0, U)], kbuf.at[slot], ksem.at[slot]).wait()

        def v_wait(slot):
            pltpu.make_async_copy(v_hbm.at[0, 0, pl.ds(0, U)], vbuf.at[slot], vsem.at[slot]).wait()

        cp_x = pltpu.make_async_copy(x_hbm.at[0], x_v, wsem.at[0])
        cp_wq = pltpu.make_async_copy(wq_hbm, wq_v, wsem.at[1])
        cp_wo = pltpu.make_async_copy(wo_hbm, wo_v, wsem.at[2])
        cp_w1 = pltpu.make_async_copy(w1_hbm, w1_v, wsem.at[3])
        cp_b1 = pltpu.make_async_copy(b1_hbm, b1_v, wsem.at[4])
        cp_w2 = pltpu.make_async_copy(w2_hbm, w2_v, wsem.at[5])
        cp_x.start()
        cp_wq.start()
        if not no_dma:
            def pre(i, c):
                k_copy(i, i).start()
                v_copy(i, i).start()
                return c
            lax.fori_loop(0, S, pre, 0)
        cp_wo.start()
        cp_w1.start()
        cp_b1.start()
        cp_w2.start()
        cp_x.wait()
        cp_wq.wait()

        row = lax.broadcasted_iota(jnp.int32, (8, DH), 0)

        def stage_a(u, slot, par):
            g = u // UPG
            q = q_v[g]
            s = _dot_nt(q, kbuf[slot])
            s_v[par] = s
            m_loc = jnp.max(s, axis=-1, keepdims=True)
            m_old = m_v[g]
            m_new = jnp.maximum(m_old, m_loc)
            m_v[g] = m_new
            alpha = jnp.exp2(m_old - m_new)
            return m_new, alpha

        def stage_b(u, slot, par, m_new, alpha):
            g = u // UPG
            s = s_v[par]
            p = jnp.exp2(s - m_new[:, 0:1])
            pv = _dot(p.astype(jnp.bfloat16), vbuf[slot])
            lsum = p[:, 0:128]
            for j in range(1, U // 128):
                lsum = lsum + p[:, j * 128:(j + 1) * 128]
            l_v[g] = l_v[g] * alpha + lsum
            acc_v[g] = acc_v[g] * alpha + pv

        x0 = x_v[...].astype(jnp.float32)

        def layer(L, x):
            xn = _ln(x).astype(jnp.bfloat16)
            xn8 = jnp.broadcast_to(xn, (8, D))
            y = _dot(xn8, wq_v[...]) * QSCALE
            for g in range(HKV):
                qg = jnp.zeros((8, DH), jnp.float32)
                for r in range(REP):
                    h = g * REP + r
                    qg = jnp.where(row == r, y[:, h * DH:(h + 1) * DH], qg)
                q_v[g] = qg.astype(jnp.bfloat16)
                m_v[g] = jnp.full((8, DH), NEG, jnp.float32)
                l_v[g] = jnp.zeros((8, DH), jnp.float32)
                acc_v[g] = jnp.zeros((8, DH), jnp.float32)

            u0 = jnp.where(L == 0, 0, NU - S)
            slot0 = jnp.where(L == 0, 0, (NU - S) % S)
            first_wait = jnp.where(L == 0, 0, S)
            n_refill = NU - S

            def refill_unit(t):
                return jnp.where(L == 0, t + S, t)

            if not no_dma:
                @pl.when(L == 0)
                def _():
                    k_wait(slot0)
            if not no_compute:
                m_new, alpha = stage_a(u0, slot0, 0)
            else:
                m_new = alpha = jnp.zeros((8, DH), jnp.float32)
            if not no_dma:
                k_copy(refill_unit(0), slot0).start()

            def step(t, carry):
                u, slot, m_new, alpha = carry
                un = jnp.where(u + 1 == NU, 0, u + 1)
                slotn = jnp.where(slot + 1 == S, 0, slot + 1)
                par = t % 2
                if not no_dma:
                    @pl.when(t >= first_wait)
                    def _():
                        v_wait(slot)

                    @pl.when(t + 1 >= first_wait)
                    def _():
                        k_wait(slotn)
                if not no_compute:
                    stage_b(u, slot, par, m_new, alpha)
                    m_new2, alpha2 = stage_a(un, slotn, 1 - par)
                else:
                    m_new2, alpha2 = m_new, alpha
                if not no_dma:
                    @pl.when(t < n_refill)
                    def _():
                        v_copy(refill_unit(t), slot).start()

                    @pl.when(t + 1 < n_refill)
                    def _():
                        k_copy(refill_unit(t + 1), slotn).start()
                return un, slotn, m_new2, alpha2

            u, slot, m_new, alpha = lax.fori_loop(0, NU - 1, step, (u0, slot0, m_new, alpha))
            if not no_dma:
                v_wait(slot)
            if not no_compute:
                stage_b(u, slot, (NU - 1) % 2, m_new, alpha)

            @pl.when(L == 0)
            def _():
                cp_wo.wait()
                cp_w1.wait()
                cp_b1.wait()
                cp_w2.wait()

            o = jnp.zeros((8, D), jnp.float32)
            for g in range(HKV):
                lsum = jnp.sum(l_v[g], axis=-1, keepdims=True)
                og = acc_v[g] / lsum
                for r in range(REP):
                    h = g * REP + r
                    ogr = jnp.where(row == r, og, 0.0).astype(jnp.bfloat16)
                    o = o + _dot(ogr, wo_v[pl.ds(h * DH, DH), :])
            a = jnp.sum(o, axis=0, keepdims=True)
            x = x + a
            xn = _ln(x).astype(jnp.bfloat16)
            h = _dot(xn, w1_v[...]) + b1_v[...].astype(jnp.float32).reshape(1, F)
            sp = jnp.log1p(jnp.exp(-jnp.abs(h))) + jnp.where(h > 0, h, 0.0)
            act = h * jnp.tanh(sp)
            x = x + _dot(act.astype(jnp.bfloat16), w2_v[...])
            return x

        x = lax.fori_loop(0, layers, layer, x0)
        out_ref[0] = x.astype(out_ref.dtype)

    bf = jnp.bfloat16
    call = pl.pallas_call(
        kernel,
        in_specs=[pl.BlockSpec(memory_space=pl.ANY)] * 8,
        out_specs=pl.BlockSpec(memory_space=pltpu.VMEM),
        out_shape=jax.ShapeDtypeStruct((1, 1, D), bf),
        scratch_shapes=[
            pltpu.VMEM((S, U, DH), bf), pltpu.VMEM((S, U, DH), bf),
            pltpu.VMEM((D, HQ * DH), bf), pltpu.VMEM((HQ * DH, D), bf),
            pltpu.VMEM((D, F), bf), pltpu.VMEM((F, D), bf),
            pltpu.VMEM((1, D), bf), pltpu.VMEM((F,), bf),
            pltpu.VMEM((HKV, 8, DH), bf),
            pltpu.VMEM((2, 8, U), jnp.float32),
            pltpu.VMEM((HKV, 8, DH), jnp.float32), pltpu.VMEM((HKV, 8, DH), jnp.float32),
            pltpu.VMEM((HKV, 8, DH), jnp.float32),
            pltpu.SemaphoreType.DMA((S,)), pltpu.SemaphoreType.DMA((S,)),
            pltpu.SemaphoreType.DMA((6,)),
        ],
        compiler_params=pltpu.CompilerParams(vmem_limit_bytes=128 * 1024 * 1024),
    )

    return call


@jax.jit
def pallas_interleave_layers__gqa_block_cached__dense_activation_mish__decode_kernel(
    A_x, A_k_cache, A_v_cache, A_wq, A_wo, B_x, B_w1, B_b1, B_w2):
    return make_kernel()(A_x, A_k_cache, A_v_cache, A_wq, A_wo, B_w1, B_b1, B_w2)
```

```python
import functools
import numpy as np
import jax
import jax.numpy as jnp
from jax import lax
import jax.experimental.pallas as pl
import jax.experimental.pallas.tpu as pltpu

HQ, HKV, DH, SK, D, F = 32, 8, 128, 65536, 512, 1792
REP = HQ // HKV
LOG2E = float(np.log2(np.e))
QSCALE = float(DH ** -0.5 * LOG2E)
NEG = -1e30
u32 = jnp.uint32
i32 = jnp.int32
f32 = jnp.float32
bf = jnp.bfloat16
M0 = np.uint32(0x807F807F)
EM = np.uint32(0x7F807F80)


def _srl(x, n):
    return lax.shift_right_logical(x, np.uint32(n))


def _sll(x, n):
    return lax.shift_left(x, np.uint32(n))


def _sh(x, n):
    if n == 0:
        return x
    return _sll(x, n) if n > 0 else _srl(x, -n)


def _ln(x):
    m = jnp.mean(x, axis=-1, keepdims=True)
    xc = x - m
    v = jnp.mean(xc * xc, axis=-1, keepdims=True)
    return xc / jnp.sqrt(v + 1e-5)


def _dot(a, b):
    return jnp.dot(a, b, preferred_element_type=f32)


def _dot_nt(a, b):
    return lax.dot_general(a, b, (((1,), (1,)), ((), ())), preferred_element_type=f32)


def _pack_sm(a, b):
    b = b & M0
    return (a & M0) | _srl(b, 8) | _sll(b, 24)


def _unpack_sm(l):
    return l & M0, (_sll(l, 8) | _srl(l, 24)) & M0


def enc12(R, e0c):
    w = [R[:, 8 * j:8 * j + 8] for j in range(4)]
    t = [(x & EM) - e0c for x in w]
    n = _srl(t[0], 7) | _srl(t[1], 3) | _sll(t[2], 1) | _sll(t[3], 5)
    viol = t[0] | t[1] | t[2] | t[3]
    return jnp.concatenate([_pack_sm(w[0], w[1]), _pack_sm(w[2], w[3]), n], axis=1), viol


def dec12(P, e0c):
    mask = np.uint32(0x07800780)
    n = P[:, 16:24]
    s0, s1 = _unpack_sm(P[:, 0:8])
    s2, s3 = _unpack_sm(P[:, 8:16])
    e = [_sll(n, 7) & mask, _sll(n, 3) & mask, _srl(n, 1) & mask, _srl(n, 5) & mask]
    return jnp.concatenate([s + x + e0c for s, x in zip((s0, s1, s2, s3), e)], axis=1)


def enc13(R, e0c):
    w = [R[:, 8 * j:8 * j + 8] for j in range(16)]
    t = [(x & EM) - e0c for x in w]
    out = [_pack_sm(w[2 * i], w[2 * i + 1]) for i in range(8)]
    for i in range(5):
        out.append(_srl(t[3 * i], 7) | _srl(t[3 * i + 1], 2) | _sll(t[3 * i + 2], 3)
                   | (_sll(t[15], 8 - i) & np.uint32(0x80008000)))
    viol = functools.reduce(lambda a, b: a | b, t)
    return jnp.concatenate(out, axis=1), viol


def dec13(P, e0c):
    mask = np.uint32(0x0F800F80)
    sm = []
    for i in range(8):
        sm.extend(_unpack_sm(P[:, 8 * i:8 * i + 8]))
    e = []
    e15 = None
    for i in range(5):
        E = P[:, 64 + 8 * i:72 + 8 * i]
        e.extend([_sll(E, 7) & mask, _sll(E, 2) & mask, _srl(E, 3) & mask])
        b = _srl(E & np.uint32(0x80008000), 8 - i)
        e15 = b if e15 is None else (e15 | b)
    e.append(e15)
    return jnp.concatenate([s + x + e0c for s, x in zip(sm, e)], axis=1)


def make_call(U=4096, SR=4, POOL_ROWS=None, force_mode=None, use_pool=True, CH=256, EK=256):
    NCH = U // CH
    NU = HKV * SK // U
    UPG = SK // U
    RW = U // 2
    PR12 = RW * 3 // 4
    PR13 = RW * 13 // 16
    if POOL_ROWS is None:
        POOL_ROWS = 72 * PR12
    NP12 = POOL_ROWS // PR12
    NP13 = POOL_ROWS // PR13
    assert NU % SR == 0

    def kernel(x_hbm, k_hbm, v_hbm, wq_hbm, wo_hbm, w1_hbm, b1_hbm, w2_hbm, out_ref,
               kst, vst, kpool, vpool, wq_v, wo_v, w1_v, w2_v, x_v, b1_v, q_v, s_v, m_v, l_v, acc_v,
               e0_v, order_s, res_s, fmt_s, off_s, st_s, ksem, vsem, wsem):
        def kv_copies(u, slot):
            g = u // UPG
            c = u % UPG
            return (pltpu.make_async_copy(k_hbm.at[0, g, pl.ds(c * U, U)], kst.at[slot], ksem.at[slot]),
                    pltpu.make_async_copy(v_hbm.at[0, g, pl.ds(c * U, U)], vst.at[slot], vsem.at[slot]))

        def kv_start(u, slot):
            a, b = kv_copies(u, slot)
            a.start()
            b.start()

        def kv_wait(slot):
            a, b = kv_copies(0, slot)
            a.wait()
            b.wait()

        cp_x = pltpu.make_async_copy(x_hbm.at[0], x_v, wsem.at[0])
        cp_wq = pltpu.make_async_copy(wq_hbm, wq_v, wsem.at[1])
        cp_wo = pltpu.make_async_copy(wo_hbm, wo_v, wsem.at[2])
        cp_w1 = pltpu.make_async_copy(w1_hbm, w1_v, wsem.at[3])
        cp_b1 = pltpu.make_async_copy(b1_hbm, b1_v, wsem.at[4])
        cp_w2 = pltpu.make_async_copy(w2_hbm, w2_v, wsem.at[5])
        cp_x.start()
        cp_wq.start()
        for i in range(SR):
            kv_start(i, i)
        cp_wo.start()
        cp_w1.start()
        cp_b1.start()
        cp_w2.start()
        for i in range(SR):
            order_s[i] = NU - SR + i
        st_s[0] = 12
        st_s[1] = 0
        st_s[2] = SR
        st_s[3] = 0
        st_s[4] = 0
        cp_x.wait()
        cp_wq.wait()

        row = lax.broadcasted_iota(i32, (8, DH), 0)

        def attend(u, kk, vv):
            g = u // UPG
            q = q_v[g]
            mx = None
            for c in range(NCH):
                s = _dot_nt(q, kk(c))
                s_v[:, pl.ds(c * CH, CH)] = s
                for j in range(CH // 128):
                    sj = s[:, j * 128:(j + 1) * 128]
                    mx = sj if mx is None else jnp.maximum(mx, sj)
            m_old = m_v[g]
            m_new = jnp.maximum(m_old, jnp.max(mx, axis=-1, keepdims=True))
            m_v[g] = m_new
            alpha = jnp.exp2(m_old - m_new)
            pv = None
            lsum = None
            for c in range(NCH):
                p = jnp.exp2(s_v[:, pl.ds(c * CH, CH)] - m_new[:, 0:1])
                r = _dot(p.astype(bf), vv(c))
                pv = r if pv is None else pv + r
                for j in range(CH // 128):
                    pj = p[:, j * 128:(j + 1) * 128]
                    lsum = pj if lsum is None else lsum + pj
            l_v[g] = l_v[g] * alpha + lsum
            acc_v[g] = acc_v[g] * alpha + pv

        def attend_pool(idx):
            u = res_s[idx]
            mode = fmt_s[idx]
            off = pl.multiple_of(off_s[idx], 8)

            def ld12(pool, e0c, c):
                ng = CH // 64
                P = pool[pl.ds(off + c * ng * 24, ng * 24), :].reshape(ng, 24, 128)
                return pltpu.bitcast(dec12(P, e0c).reshape(CH // 2, 128), bf)

            def ld13(pool, e0c, c):
                ng = CH // 256
                P = pool[pl.ds(off + c * ng * 104, ng * 104), :].reshape(ng, 104, 128)
                return pltpu.bitcast(dec13(P, e0c).reshape(CH // 2, 128), bf)

            def ld16(pool, c):
                return pltpu.bitcast(pool[pl.ds(off + c * (CH // 2), CH // 2), :], bf)

            @pl.when(mode == 12)
            def _():
                ek, ev = e0_v[0], e0_v[1]
                attend(u, lambda c: ld12(kpool, ek, c), lambda c: ld12(vpool, ev, c))

            @pl.when(mode == 13)
            def _():
                ek, ev = e0_v[0], e0_v[1]
                attend(u, lambda c: ld13(kpool, ek, c), lambda c: ld13(vpool, ev, c))

            @pl.when(mode == 16)
            def _():
                attend(u, lambda c: ld16(kpool, c), lambda c: ld16(vpool, c))

        def exp_range(st, slot):
            def body(c, carry):
                mx, mn = carry
                w = pltpu.bitcast(st[slot, pl.ds(pl.multiple_of(c * 256, 256), 256), :], u32).reshape(16, 8, 128)
                lo = (_srl(w, 7) & np.uint32(0xFF)).astype(i32)
                hi = (_srl(w, 23) & np.uint32(0xFF)).astype(i32)
                mx = jnp.maximum(mx, jnp.max(jnp.maximum(lo, hi), axis=0))
                mn = jnp.minimum(mn, jnp.min(jnp.minimum(lo, hi), axis=0))
                return mx, mn
            mx, mn = lax.fori_loop(0, U // 256, body,
                                   (jnp.zeros((8, 128), i32), jnp.full((8, 128), 255, i32)))
            return jnp.max(mx.astype(f32)).astype(i32), jnp.min(mn.astype(f32)).astype(i32)

        def choose_format():
            kmx, kmn = exp_range(kst, 0)
            vmx, vmn = exp_range(vst, 0)
            span = jnp.maximum(kmx - kmn, vmx - vmn) + 1
            mode = jnp.where(span <= 12, 12, 13).astype(i32)
            if force_mode is not None:
                mode = jnp.full_like(mode, force_mode)
            width = jnp.where(mode == 12, 16, 32)
            st_s[0] = mode
            for i, mx in enumerate((kmx, vmx)):
                top = jnp.minimum(mx + 2, 255)
                base = jnp.maximum(top - (width - 1), 0)
                e0 = (base * (128 * 0x10001)).astype(u32)
                e0_v[i] = jnp.full((8, 128), e0, u32)

        def encode(t, slot):
            mode = st_s[0]
            idx = st_s[1]
            top = pl.multiple_of(st_s[3], 8)
            st_s[4] = 0

            def commit(fmt, rows):
                res_s[idx] = t
                fmt_s[idx] = fmt
                off_s[idx] = top
                st_s[1] = idx + 1
                st_s[3] = top + rows
                st_s[4] = 1

            def finish(viol, mask, fmt, rows):
                bad = (viol & mask) != 0
                nbad = jnp.max(bad.astype(f32))

                @pl.when(nbad == 0.0)
                def _():
                    commit(fmt, rows)

            def enc_loop(enc, keys, rows_in, rows_out):
                def body(c, viol):
                    for st, pool, i in ((kst, kpool, 0), (vst, vpool, 1)):
                        R = pltpu.bitcast(st[slot, pl.ds(pl.multiple_of(c * keys, keys), keys), :], u32)
                        P, vi = enc(R.reshape(-1, rows_in, 128), e0_v[i])
                        n = P.shape[0]
                        pool[pl.ds(pl.multiple_of(top + c * (n * rows_out), 8), n * rows_out), :] = (
                            P.reshape(n * rows_out, 128))
                        for j in range(n):
                            viol = viol | vi[j]
                    return viol
                return lax.fori_loop(0, U // keys, body, jnp.zeros((8, 128), u32))

            @pl.when(jnp.logical_and(top + PR12 <= POOL_ROWS, mode == 12))
            def _():
                finish(enc_loop(enc12, EK, 32, 24), np.uint32(0xF87FF87F), 12, PR12)

            @pl.when(jnp.logical_and(top + PR13 <= POOL_ROWS, mode == 13))
            def _():
                finish(enc_loop(enc13, EK, 128, 104), np.uint32(0xF07FF07F), 13, PR13)

            @pl.when(jnp.logical_and(st_s[4] == 0, top + RW <= POOL_ROWS))
            def _():
                def body(c, carry):
                    for st, pool in ((kst, kpool), (vst, vpool)):
                        pool[pl.ds(pl.multiple_of(top + c * (EK // 2), 8), EK // 2), :] = pltpu.bitcast(
                            st[slot, pl.ds(pl.multiple_of(c * EK, EK), EK), :], u32)
                    return carry
                lax.fori_loop(0, U // EK, body, 0)
                commit(16, RW)

            @pl.when(st_s[4] == 0)
            def _():
                order_s[st_s[2]] = t
                st_s[2] = st_s[2] + 1

        x0 = x_v[...].astype(f32)

        def layer(L, x):
            xn = _ln(x).astype(bf)
            xn8 = jnp.broadcast_to(xn, (8, D))
            y = _dot(xn8, wq_v[...]) * QSCALE
            for g in range(HKV):
                qg = jnp.zeros((8, DH), f32)
                for r in range(REP):
                    h = g * REP + r
                    qg = jnp.where(row == r, y[:, h * DH:(h + 1) * DH], qg)
                q_v[g] = qg.astype(bf)
                m_v[g] = jnp.full((8, DH), NEG, f32)
                l_v[g] = jnp.zeros((8, DH), f32)
                acc_v[g] = jnp.zeros((8, DH), f32)

            first = L == 0
            n_raw = jnp.where(first, NU, st_s[2])
            n_pool = jnp.where(first, 0, st_s[1])

            def unit_of(j):
                return jnp.where(first, j, order_s[jnp.where(first, 0, j)])

            def step(j, done):
                slot = j % SR
                left = n_pool - done
                rem = n_raw - j
                cnt = jnp.where(j < SR, jnp.where(rem == 1, left, 0), (left + rem - 1) // rem)
                if use_pool:
                    def pool_step(i, c):
                        attend_pool(done + i)
                        return c
                    lax.fori_loop(0, cnt, pool_step, 0)

                @pl.when(jnp.logical_or(first, j >= SR))
                def _():
                    kv_wait(slot)

                u = unit_of(j)
                attend(u, lambda c: kst[slot, pl.ds(c * CH, CH), :], lambda c: vst[slot, pl.ds(c * CH, CH), :])

                if use_pool:
                    @pl.when(jnp.logical_and(first, j == 0))
                    def _():
                        choose_format()

                    @pl.when(jnp.logical_and(first, j < NU - SR))
                    def _():
                        encode(j, slot)
                else:
                    @pl.when(jnp.logical_and(first, j < NU - SR))
                    def _():
                        order_s[st_s[2]] = j
                        st_s[2] = st_s[2] + 1

                @pl.when(j + SR < n_raw)
                def _():
                    kv_start(unit_of(j + SR), slot)
                return done + cnt

            lax.fori_loop(0, n_raw, step, 0)

            @pl.when(first)
            def _():
                cp_wo.wait()
                cp_w1.wait()
                cp_b1.wait()
                cp_w2.wait()

            o = jnp.zeros((8, D), f32)
            for g in range(HKV):
                lsum = jnp.sum(l_v[g], axis=-1, keepdims=True)
                og = acc_v[g] / lsum
                for r in range(REP):
                    h = g * REP + r
                    ogr = jnp.where(row == r, og, 0.0).astype(bf)
                    o = o + _dot(ogr, wo_v[pl.ds(h * DH, DH), :])
            a = jnp.sum(o, axis=0, keepdims=True)
            x = x + a
            xn = _ln(x).astype(bf)
            h = _dot(xn, w1_v[...]) + b1_v[...].astype(f32).reshape(1, F)
            sp = jnp.log1p(jnp.exp(-jnp.abs(h))) + jnp.where(h > 0, h, 0.0)
            act = h * jnp.tanh(sp)
            x = x + _dot(act.astype(bf), w2_v[...])
            return x

        x = lax.fori_loop(0, 2, layer, x0)
        out_ref[0] = x.astype(out_ref.dtype)

    call = pl.pallas_call(
        kernel,
        in_specs=[pl.BlockSpec(memory_space=pl.ANY)] * 8,
        out_specs=pl.BlockSpec(memory_space=pltpu.VMEM),
        out_shape=jax.ShapeDtypeStruct((1, 1, D), bf),
        scratch_shapes=[
            pltpu.VMEM((SR, U, DH), bf), pltpu.VMEM((SR, U, DH), bf),
            pltpu.VMEM((POOL_ROWS, 128), u32), pltpu.VMEM((POOL_ROWS, 128), u32),
            pltpu.VMEM((D, HQ * DH), bf), pltpu.VMEM((HQ * DH, D), bf),
            pltpu.VMEM((D, F), bf), pltpu.VMEM((F, D), bf),
            pltpu.VMEM((1, D), bf), pltpu.VMEM((F,), bf),
            pltpu.VMEM((HKV, 8, DH), bf),
            pltpu.VMEM((8, U), f32),
            pltpu.VMEM((HKV, 8, DH), f32), pltpu.VMEM((HKV, 8, DH), f32),
            pltpu.VMEM((HKV, 8, DH), f32),
            pltpu.VMEM((2, 8, 128), u32),
            pltpu.SMEM((NU,), i32), pltpu.SMEM((NU,), i32), pltpu.SMEM((NU,), i32),
            pltpu.SMEM((NU,), i32), pltpu.SMEM((8,), i32),
            pltpu.SemaphoreType.DMA((SR,)), pltpu.SemaphoreType.DMA((SR,)),
            pltpu.SemaphoreType.DMA((6,)),
        ],
        compiler_params=pltpu.CompilerParams(vmem_limit_bytes=128 * 1024 * 1024),
    )
    return call


@jax.jit
def pallas_interleave_layers__gqa_block_cached__dense_activation_mish__decode_kernel(
        A_x, A_k_cache, A_v_cache, A_wq, A_wo, B_x, B_w1, B_b1, B_w2):
    del B_x
    return make_call()(A_x, A_k_cache, A_v_cache, A_wq, A_wo, B_w1, B_b1, B_w2)
```

```python
import functools
import numpy as np
import jax
import jax.numpy as jnp
from jax import lax
import jax.experimental.pallas as pl
import jax.experimental.pallas.tpu as pltpu

HQ, HKV, DH, SK, D, F = 32, 8, 128, 65536, 512, 1792
REP = HQ // HKV
LOG2E = float(np.log2(np.e))
QSCALE = float(DH ** -0.5 * LOG2E)
NEG = -1e30
u32 = jnp.uint32
i32 = jnp.int32
f32 = jnp.float32
bf = jnp.bfloat16
M0 = np.uint32(0x807F807F)
EM = np.uint32(0x7F807F80)


def _srl(x, n):
    return lax.shift_right_logical(x, np.uint32(n))


def _sll(x, n):
    return lax.shift_left(x, np.uint32(n))


def _sh(x, n):
    if n == 0:
        return x
    return _sll(x, n) if n > 0 else _srl(x, -n)


def _ln(x):
    m = jnp.mean(x, axis=-1, keepdims=True)
    xc = x - m
    v = jnp.mean(xc * xc, axis=-1, keepdims=True)
    return xc / jnp.sqrt(v + 1e-5)


def _dot(a, b):
    return jnp.dot(a, b, preferred_element_type=f32)


def _dot_nt(a, b):
    return lax.dot_general(a, b, (((1,), (1,)), ((), ())), preferred_element_type=f32)


def _pack_sm(a, b):
    b = b & M0
    return (a & M0) | _srl(b, 8) | _sll(b, 24)


def _unpack_sm(l):
    return l & M0, (_sll(l, 8) | _srl(l, 24)) & M0


def enc12(R, e0c):
    w = [R[:, 8 * j:8 * j + 8] for j in range(4)]
    t = [(x & EM) - e0c for x in w]
    n = _srl(t[0], 7) | _srl(t[1], 3) | _sll(t[2], 1) | _sll(t[3], 5)
    viol = t[0] | t[1] | t[2] | t[3]
    return jnp.concatenate([_pack_sm(w[0], w[1]), _pack_sm(w[2], w[3]), n], axis=1), viol


def dec12(P, e0c):
    mask = np.uint32(0x07800780)
    n = P[:, 16:24]
    s0, s1 = _unpack_sm(P[:, 0:8])
    s2, s3 = _unpack_sm(P[:, 8:16])
    e = [_sll(n, 7) & mask, _sll(n, 3) & mask, _srl(n, 1) & mask, _srl(n, 5) & mask]
    return jnp.concatenate([s + x + e0c for s, x in zip((s0, s1, s2, s3), e)], axis=1)


def enc13(R, e0c):
    w = [R[:, 8 * j:8 * j + 8] for j in range(16)]
    t = [(x & EM) - e0c for x in w]
    out = [_pack_sm(w[2 * i], w[2 * i + 1]) for i in range(8)]
    for i in range(5):
        out.append(_srl(t[3 * i], 7) | _srl(t[3 * i + 1], 2) | _sll(t[3 * i + 2], 3)
                   | (_sll(t[15], 8 - i) & np.uint32(0x80008000)))
    viol = functools.reduce(lambda a, b: a | b, t)
    return jnp.concatenate(out, axis=1), viol


def dec13(P, e0c):
    mask = np.uint32(0x0F800F80)
    sm = []
    for i in range(8):
        sm.extend(_unpack_sm(P[:, 8 * i:8 * i + 8]))
    e = []
    e15 = None
    for i in range(5):
        E = P[:, 64 + 8 * i:72 + 8 * i]
        e.extend([_sll(E, 7) & mask, _sll(E, 2) & mask, _srl(E, 3) & mask])
        b = _srl(E & np.uint32(0x80008000), 8 - i)
        e15 = b if e15 is None else (e15 | b)
    e.append(e15)
    return jnp.concatenate([s + x + e0c for s, x in zip(sm, e)], axis=1)


def make_call(U=4096, SR=4, CH=256, EK=256):
    NCH = U // CH
    NU = HKV * SK // U
    UPG = SK // U
    RW = U // 2
    PR12 = RW * 3 // 4
    PR13 = RW * 13 // 16
    POOL_ROWS = 72 * PR12
    assert NU % SR == 0

    def kernel(x_hbm, k_hbm, v_hbm, wq_hbm, wo_hbm, w1_hbm, b1_hbm, w2_hbm, out_ref,
               kst, vst, kpool, vpool, wq_v, wo_v, w1_v, w2_v, x_v, b1_v, q_v, s_v, m_v, l_v, acc_v,
               e0_v, xn_v, o_v, order_s, res_s, fmt_s, off_s, cnt_s, st_s, ksem, vsem, wsem, qsem):
        def k_copy(u, slot):
            return pltpu.make_async_copy(
                k_hbm.at[0, u // UPG, pl.ds((u % UPG) * U, U)], kst.at[slot], ksem.at[slot])

        def v_copy(u, slot):
            return pltpu.make_async_copy(
                v_hbm.at[0, u // UPG, pl.ds((u % UPG) * U, U)], vst.at[slot], vsem.at[slot])

        cp_x = pltpu.make_async_copy(x_hbm.at[0], x_v, wsem.at[0])
        cp_wq = [pltpu.make_async_copy(wq_hbm.at[:, pl.ds(g * REP * DH, REP * DH)], wq_v.at[g], qsem.at[g])
                 for g in range(HKV)]
        cp_wo = pltpu.make_async_copy(wo_hbm, wo_v, wsem.at[2])
        cp_w1 = pltpu.make_async_copy(w1_hbm, w1_v, wsem.at[3])
        cp_b1 = pltpu.make_async_copy(b1_hbm, b1_v, wsem.at[4])
        cp_w2 = pltpu.make_async_copy(w2_hbm, w2_v, wsem.at[5])
        cp_x.start()
        for c in cp_wq:
            c.start()
        for i in range(SR):
            k_copy(i, i).start()
            v_copy(i, i).start()
        cp_wo.start()
        cp_w1.start()
        cp_b1.start()
        cp_w2.start()
        for i in range(SR):
            order_s[i] = NU - SR + i
        st_s[0] = 12
        st_s[1] = 0
        st_s[2] = SR
        st_s[3] = 0
        st_s[4] = 0
        cp_x.wait()
        for c in cp_wq:
            c.wait()

        row = lax.broadcasted_iota(i32, (8, DH), 0)

        def attend(u, kk, vv, mid=None):
            g = u // UPG
            q = q_v[g]
            mx = None
            for c in range(NCH):
                s = _dot_nt(q, kk(c))
                s_v[:, pl.ds(c * CH, CH)] = s
                for j in range(CH // 128):
                    sj = s[:, j * 128:(j + 1) * 128]
                    mx = sj if mx is None else jnp.maximum(mx, sj)
            m_old = m_v[g]
            m_new = jnp.maximum(m_old, jnp.max(mx, axis=-1, keepdims=True))
            m_v[g] = m_new
            alpha = jnp.exp2(m_old - m_new)
            if mid is not None:
                mid()
            pv = None
            lsum = None
            for c in range(NCH):
                p = jnp.exp2(s_v[:, pl.ds(c * CH, CH)] - m_new[:, 0:1])
                r = _dot(p.astype(bf), vv(c))
                pv = r if pv is None else pv + r
                for j in range(CH // 128):
                    pj = p[:, j * 128:(j + 1) * 128]
                    lsum = pj if lsum is None else lsum + pj
            l_v[g] = l_v[g] * alpha + lsum
            acc_v[g] = acc_v[g] * alpha + pv

        def attend_pool(idx):
            u = res_s[idx]
            mode = fmt_s[idx]
            off = pl.multiple_of(off_s[idx], 8)

            def ld12(pool, e0c, c):
                ng = CH // 64
                P = pool[pl.ds(off + c * ng * 24, ng * 24), :].reshape(ng, 24, 128)
                return pltpu.bitcast(dec12(P, e0c).reshape(CH // 2, 128), bf)

            def ld13(pool, e0c, c):
                ng = CH // 256
                P = pool[pl.ds(off + c * ng * 104, ng * 104), :].reshape(ng, 104, 128)
                return pltpu.bitcast(dec13(P, e0c).reshape(CH // 2, 128), bf)

            def ld16(pool, c):
                return pltpu.bitcast(pool[pl.ds(off + c * (CH // 2), CH // 2), :], bf)

            @pl.when(mode == 12)
            def _():
                ek, ev = e0_v[0], e0_v[1]
                attend(u, lambda c: ld12(kpool, ek, c), lambda c: ld12(vpool, ev, c))

            @pl.when(mode == 13)
            def _():
                ek, ev = e0_v[0], e0_v[1]
                attend(u, lambda c: ld13(kpool, ek, c), lambda c: ld13(vpool, ev, c))

            @pl.when(mode == 16)
            def _():
                attend(u, lambda c: ld16(kpool, c), lambda c: ld16(vpool, c))

        def exp_range(st, slot):
            def body(c, carry):
                mx, mn = carry
                w = pltpu.bitcast(st[slot, pl.ds(pl.multiple_of(c * 256, 256), 256), :], u32).reshape(16, 8, 128)
                lo = (_srl(w, 7) & np.uint32(0xFF)).astype(i32)
                hi = (_srl(w, 23) & np.uint32(0xFF)).astype(i32)
                mx = jnp.maximum(mx, jnp.max(jnp.maximum(lo, hi), axis=0))
                mn = jnp.minimum(mn, jnp.min(jnp.minimum(lo, hi), axis=0))
                return mx, mn
            mx, mn = lax.fori_loop(0, U // 256, body,
                                   (jnp.zeros((8, 128), i32), jnp.full((8, 128), 255, i32)))
            return jnp.max(mx.astype(f32)).astype(i32), jnp.min(mn.astype(f32)).astype(i32)

        def choose_format():
            kmx, kmn = exp_range(kst, 0)
            vmx, vmn = exp_range(vst, 0)
            span = jnp.maximum(kmx - kmn, vmx - vmn) + 1
            mode = jnp.where(span <= 12, 12, 13).astype(i32)
            width = jnp.where(mode == 12, 16, 32)
            st_s[0] = mode
            for i, mx in enumerate((kmx, vmx)):
                top = jnp.minimum(mx + 2, 255)
                base = jnp.maximum(top - (width - 1), 0)
                e0 = (base * (128 * 0x10001)).astype(u32)
                e0_v[i] = jnp.full((8, 128), e0, u32)

        def encode(t, slot):
            mode = st_s[0]
            idx = st_s[1]
            top = pl.multiple_of(st_s[3], 8)
            st_s[4] = 0

            def commit(fmt, rows):
                res_s[idx] = t
                fmt_s[idx] = fmt
                off_s[idx] = top
                st_s[1] = idx + 1
                st_s[3] = top + rows
                st_s[4] = 1

            def finish(viol, mask, fmt, rows):
                bad = (viol & mask) != 0
                nbad = jnp.max(bad.astype(f32))

                @pl.when(nbad == 0.0)
                def _():
                    commit(fmt, rows)

            def enc_loop(enc, keys, rows_in, rows_out):
                def body(c, viol):
                    for st, pool, i in ((kst, kpool, 0), (vst, vpool, 1)):
                        R = pltpu.bitcast(st[slot, pl.ds(pl.multiple_of(c * keys, keys), keys), :], u32)
                        P, vi = enc(R.reshape(-1, rows_in, 128), e0_v[i])
                        n = P.shape[0]
                        pool[pl.ds(pl.multiple_of(top + c * (n * rows_out), 8), n * rows_out), :] = (
                            P.reshape(n * rows_out, 128))
                        for j in range(n):
                            viol = viol | vi[j]
                    return viol
                return lax.fori_loop(0, U // keys, body, jnp.zeros((8, 128), u32))

            @pl.when(jnp.logical_and(top + PR12 <= POOL_ROWS, mode == 12))
            def _():
                finish(enc_loop(enc12, EK, 32, 24), np.uint32(0xF87FF87F), 12, PR12)

            @pl.when(jnp.logical_and(top + PR13 <= POOL_ROWS, mode == 13))
            def _():
                finish(enc_loop(enc13, EK, 128, 104), np.uint32(0xF07FF07F), 13, PR13)

            @pl.when(jnp.logical_and(st_s[4] == 0, top + RW <= POOL_ROWS))
            def _():
                def body(c, carry):
                    for st, pool in ((kst, kpool), (vst, vpool)):
                        pool[pl.ds(pl.multiple_of(top + c * (EK // 2), 8), EK // 2), :] = pltpu.bitcast(
                            st[slot, pl.ds(pl.multiple_of(c * EK, EK), EK), :], u32)
                    return carry
                lax.fori_loop(0, U // EK, body, 0)
                commit(16, RW)

            @pl.when(st_s[4] == 0)
            def _():
                order_s[st_s[2]] = t
                st_s[2] = st_s[2] + 1

        def project_q(g):
            y = _dot(xn_v[...], wq_v[g]) * QSCALE
            qg = jnp.zeros((8, DH), f32)
            for r in range(REP):
                qg = jnp.where(row == r, y[:, r * DH:(r + 1) * DH], qg)
            q_v[g] = qg.astype(bf)

        def unit_done(u):
            g = u // UPG
            left = cnt_s[g] - 1
            cnt_s[g] = left

            @pl.when(left == 0)
            def _():
                og = acc_v[g] / jnp.sum(l_v[g], axis=-1, keepdims=True)
                o = o_v[...]
                for r in range(REP):
                    ogr = jnp.where(row == r, og, 0.0).astype(bf)
                    o = o + _dot(ogr, wo_v[pl.ds(pl.multiple_of((g * REP + r) * DH, DH), DH), :])
                o_v[...] = o

        x0 = x_v[...].astype(f32)

        def layer(L, x):
            first = L == 0
            xn_v[...] = jnp.broadcast_to(_ln(x).astype(bf), (8, D))
            for g in range(HKV):
                m_v[g] = jnp.full((8, DH), NEG, f32)
                l_v[g] = jnp.zeros((8, DH), f32)
                acc_v[g] = jnp.zeros((8, DH), f32)
                cnt_s[g] = UPG
            o_v[...] = jnp.zeros((8, D), f32)
            project_q(jnp.where(first, 0, HKV - 1))

            n_raw = jnp.where(first, NU, st_s[2])
            n_pool = jnp.where(first, 0, st_s[1])

            def unit_of(j):
                return jnp.where(first, j, order_s[jnp.where(first, 0, j)])

            def step(j, done):
                slot = j % SR
                left = n_pool - done
                rem = n_raw - j
                cnt = jnp.where(j < SR, jnp.where(rem == 1, left, 0), (left + rem - 1) // rem)
                def pool_step(i, c):
                    attend_pool(done + i)
                    unit_done(res_s[done + i])
                    return c
                lax.fori_loop(0, cnt, pool_step, 0)

                need_wait = jnp.logical_or(first, j >= SR)
                need_fill = j + SR < n_raw
                u_next = unit_of(jnp.where(need_fill, j + SR, 0))

                @pl.when(need_wait)
                def _():
                    k_copy(0, slot).wait()

                def mid():
                    @pl.when(need_wait)
                    def _():
                        v_copy(0, slot).wait()

                    @pl.when(jnp.logical_and(need_fill, jnp.logical_not(first)))
                    def _():
                        k_copy(u_next, slot).start()

                u = unit_of(j)
                attend(u, lambda c: kst[slot, pl.ds(c * CH, CH), :], lambda c: vst[slot, pl.ds(c * CH, CH), :], mid)

                @pl.when(jnp.logical_and(first, j == 0))
                def _():
                    choose_format()

                @pl.when(jnp.logical_and(first, j < NU - SR))
                def _():
                    encode(j, slot)

                @pl.when(jnp.logical_and(need_fill, first))
                def _():
                    k_copy(u_next, slot).start()

                @pl.when(need_fill)
                def _():
                    v_copy(u_next, slot).start()

                @pl.when(j == 0)
                def _():
                    def body(g, c):
                        project_q(g)
                        return c
                    lax.fori_loop(0, HKV, body, 0)

                    @pl.when(first)
                    def _():
                        cp_wo.wait()
                        cp_w1.wait()
                        cp_b1.wait()
                        cp_w2.wait()

                unit_done(u)
                return done + cnt

            lax.fori_loop(0, n_raw, step, 0)

            a = jnp.sum(o_v[...], axis=0, keepdims=True)
            x = x + a
            xn = _ln(x).astype(bf)
            h = _dot(xn, w1_v[...]) + b1_v[...].astype(f32).reshape(1, F)
            sp = jnp.log1p(jnp.exp(-jnp.abs(h))) + jnp.where(h > 0, h, 0.0)
            act = h * jnp.tanh(sp)
            x = x + _dot(act.astype(bf), w2_v[...])
            return x

        x = lax.fori_loop(0, 2, layer, x0)
        out_ref[0] = x.astype(out_ref.dtype)

    call = pl.pallas_call(
        kernel,
        in_specs=[pl.BlockSpec(memory_space=pl.ANY)] * 8,
        out_specs=pl.BlockSpec(memory_space=pltpu.VMEM),
        out_shape=jax.ShapeDtypeStruct((1, 1, D), bf),
        scratch_shapes=[
            pltpu.VMEM((SR, U, DH), bf), pltpu.VMEM((SR, U, DH), bf),
            pltpu.VMEM((POOL_ROWS, 128), u32), pltpu.VMEM((POOL_ROWS, 128), u32),
            pltpu.VMEM((HKV, D, REP * DH), bf), pltpu.VMEM((HQ * DH, D), bf),
            pltpu.VMEM((D, F), bf), pltpu.VMEM((F, D), bf),
            pltpu.VMEM((1, D), bf), pltpu.VMEM((F,), bf),
            pltpu.VMEM((HKV, 8, DH), bf),
            pltpu.VMEM((8, U), f32),
            pltpu.VMEM((HKV, 8, DH), f32), pltpu.VMEM((HKV, 8, DH), f32),
            pltpu.VMEM((HKV, 8, DH), f32),
            pltpu.VMEM((2, 8, 128), u32), pltpu.VMEM((8, D), bf), pltpu.VMEM((8, D), f32),
            pltpu.SMEM((NU,), i32), pltpu.SMEM((NU,), i32), pltpu.SMEM((NU,), i32),
            pltpu.SMEM((NU,), i32), pltpu.SMEM((HKV,), i32), pltpu.SMEM((8,), i32),
            pltpu.SemaphoreType.DMA((SR,)), pltpu.SemaphoreType.DMA((SR,)),
            pltpu.SemaphoreType.DMA((6,)), pltpu.SemaphoreType.DMA((HKV,)),
        ],
        compiler_params=pltpu.CompilerParams(vmem_limit_bytes=128 * 1024 * 1024),
    )
    return call


@jax.jit
def pallas_interleave_layers__gqa_block_cached__dense_activation_mish__decode_kernel(
        A_x, A_k_cache, A_v_cache, A_wq, A_wo, B_x, B_w1, B_b1, B_w2):
    del B_x
    return make_call()(A_x, A_k_cache, A_v_cache, A_wq, A_wo, B_w1, B_b1, B_w2)
```
